```python
import jax
import jax.numpy as jnp

def _softmax(x, axis=-1):
    return jax.nn.softmax(x, axis=axis)
def _gelu(x):
    return jax.nn.gelu(x, approximate=True)
def _silu(x):
    return jax.nn.silu(x)
def _sigmoid(x):
    return jax.nn.sigmoid(x)
def _layernorm(x, axis=-1, eps=1e-5):
    m = jnp.mean(x, axis=axis, keepdims=True)
    v = jnp.var(x, axis=axis, keepdims=True)
    return (x - m) / jnp.sqrt(v + eps)
def _scatter_add(tgt, idx, src, axis=0):
    return tgt.at[idx].add(src)
def _segment_sum(src, seg, n):
    return jax.ops.segment_sum(src, seg, n)
class _Rng:
    def __init__(self, key):
        self._k = key
    def _next(self):
        self._k, sub = jax.random.split(self._k)
        return sub
    def normal(self, shape):
        return jax.random.normal(self._next(), shape, dtype=jnp.bfloat16)
    def randint(self, lo, hi, shape):
        return jax.random.randint(self._next(), shape, lo, hi, dtype=jnp.int32)
    def uniform(self, shape, lo=0.0, hi=1.0):
        return jax.random.uniform(self._next(), shape, jnp.bfloat16, lo, hi)
    def permutation(self, n):
        return jax.random.permutation(self._next(), n)


kernel_name = 'gated_mix__sliding_block_cached__dense_activation_gelu__decode'

def setup_inputs():
    _rng = _Rng(jax.random.key(int.from_bytes(__import__("os").urandom(4), "little")))
    _w = (lambda a: (lambda t: t.astype(jnp.bfloat16) if jnp.issubdtype(t.dtype, jnp.floating) else t)(jnp.asarray(a)))
    def _A_setup():
        B, Sq, D = 1, 1, 640
        Hq, Hkv, Sk, Dh = 32, 32, 32768, 192
        assert Hq % Hkv == 0, (Hq, Hkv)
        return {
            "x": _w((lambda *s: _rng.normal(s) * 0.05)(B, Sq, D)),
            "k_cache": _w((lambda *s: _rng.normal(s) * 0.05)(B, Hkv, Sk, Dh)),
            "v_cache": _w((lambda *s: _rng.normal(s) * 0.05)(B, Hkv, Sk, Dh)),
            "wq": _w((lambda *s: _rng.normal(s) * 0.05)(D, Hq * Dh) * (D ** -0.5)),
            "wo": _w((lambda *s: _rng.normal(s) * 0.05)(Hq * Dh, D) * ((Hq * Dh) ** -0.5)),
        }
    _A_in = _A_setup()

    def _B_setup():
        B, S, D, F = 1, 1, 640, 1536
        return {
            "x": _w((lambda *s: _rng.normal(s) * 0.05)(B, S, D)),
            "w1": _w((lambda *s: _rng.normal(s) * 0.05)(D, F) * (D ** -0.5)),
            "b1": _w((lambda *s: _rng.normal(s) * 0.05)(F) * 0.01),
            "w2": _w((lambda *s: _rng.normal(s) * 0.05)(F, D) * (F ** -0.5)),
            "b2": _w((lambda *s: _rng.normal(s) * 0.05)(D) * 0.01),
        }
    _B_in = _B_setup()

    return {
        "A_x": _A_in["x"],
        "A_k_cache": _A_in["k_cache"],
        "A_v_cache": _A_in["v_cache"],
        "A_wq": _A_in["wq"],
        "A_wo": _A_in["wo"],
        "B_x": _B_in["x"],
        "B_w1": _B_in["w1"],
        "B_b1": _B_in["b1"],
        "B_w2": _B_in["w2"],
        "B_b2": _B_in["b2"],
        "gate_w": _w((lambda *s: _rng.normal(s) * 0.05)(640)),
    }

def reference(A_x, A_k_cache, A_v_cache, A_wq, A_wo, B_x, B_w1, B_b1, B_w2, B_b2, gate_w):
    def _A_ref(x, k_cache, v_cache, wq, wo):
        B, Sq, D = x.shape
        Hq, Dh = 32, 192
        Hkv, Sk = k_cache.shape[1], k_cache.shape[2]
        W = min(4096, max(256, Sk // 4))
        rep = Hq // Hkv
        q = (lambda x, *d: x.transpose(*d))((x @ wq).reshape(B, Sq, Hq, Dh), 0, 2, 1, 3)
        k = jnp.repeat(k_cache[:, :, Sk - W:, :], rep, axis=1)
        v = jnp.repeat(v_cache[:, :, Sk - W:, :], rep, axis=1)
        scores = jnp.einsum("bhqd,bhkd->bhqk", q, k) * (Dh ** -0.5)
        p = _softmax(scores, axis=-1)
        o = jnp.einsum("bhqk,bhkd->bhqd", p, v)
        return (lambda x, *d: x.transpose(*d))(o, 0, 2, 1, 3).reshape(B, Sq, Hq * Dh) @ wo

    def _B_ref(x, w1, b1, w2, b2):
        h = jnp.einsum("bsd,df->bsf", x, w1) + b1
        h = _gelu(h)
        return jnp.einsum("bsf,fd->bsd", h, w2) + b2

    x = A_x
    g = _sigmoid((x * gate_w).sum(-1, keepdims=True))
    a = _A_ref(x, A_k_cache, A_v_cache, A_wq, A_wo)
    b = _B_ref(x, B_w1, B_b1, B_w2, B_b2)
    return g * a + (1 - g) * b
```

```python
import functools
import jax
import jax.numpy as jnp
from jax import lax
import jax.experimental.pallas as pl
import jax.experimental.pallas.tpu as pltpu

HQ, DH = 32, 192
GH = 8
GR = GH * DH
NT_ = GR // 128
CW = 2048
JR = 8
F32, BF16 = jnp.float32, jnp.bfloat16


def _gelu(x):
    return jax.nn.gelu(x, approximate=True)


def make_kernel(Sk, W, D_MODEL, F, *, D=4, NS=8, pat="0111"):
    NG = HQ // GH
    NC = W // CW
    KT = D_MODEL // 128
    QC = HQ * DH // CW
    n_wq = KT * QC
    WB = 384
    n_w2 = F // WB
    n_wo = HQ * DH // WB
    scale = DH ** -0.5
    assert D % 2 == 0 and NC == 2 and NS & (NS - 1) == 0 and NS > D

    def prio(n):
        return int(pat[n % len(pat)])

    def kernel(ax_hbm, k_hbm, v_hbm, wq_hbm, wo_hbm, w1_hbm, b1_hbm, w2_hbm, b2_hbm, gw_hbm,
               o_ref,
               ring, wq_buf, w1_buf, w2_buf, wo_buf,
               ax_s, b1_s, b2_s, gw_s,
               xa_scr, q_scr, h_scr, s_scr, p_scr, o_scr, il_scr,
               ring_sem, wq_sem, w1_sem, w2_sem, wo_sem, small_sem):

        def issue_kv(src, g, rt, c, slot):
            for i in range(128 // JR):
                r0 = pl.multiple_of(g * GR + rt * 128 + i * JR, JR)
                c0 = Sk - W + c * CW
                pltpu.make_async_copy(src.at[pl.ds(r0, JR), pl.ds(c0, CW)],
                                      ring.at[slot, pl.ds(i * JR, JR), :],
                                      ring_sem.at[slot]).start(priority=prio(i))

        def issue_wq(t):
            c = t // KT
            kt = t - c * KT
            for i in range(128 // JR):
                r0 = pl.multiple_of(kt * 128 + i * JR, JR)
                c0 = pl.multiple_of(c * CW, CW)
                pltpu.make_async_copy(wq_hbm.at[pl.ds(r0, JR), pl.ds(c0, CW)],
                                      wq_buf.at[t, pl.ds(i * JR, JR), :],
                                      wq_sem.at[t]).start(priority=prio(i))

        def issue_w1(kt):
            for i in range(128 // JR):
                r0 = pl.multiple_of(kt * 128 + i * JR, JR)
                pltpu.make_async_copy(w1_hbm.at[pl.ds(r0, JR), :],
                                      w1_buf.at[kt, pl.ds(i * JR, JR), :],
                                      w1_sem.at[kt]).start(priority=prio(i))

        def issue_w(src, buf, sem, j):
            jr = WB // 16
            for i in range(16):
                r0 = pl.multiple_of(j * WB + i * jr, 8)
                pltpu.make_async_copy(src.at[pl.ds(r0, jr), :],
                                      buf.at[j, pl.ds(i * jr, jr), :],
                                      sem.at[j]).start(priority=prio(i))

        def wait_buf(buf, sem, j):
            pltpu.make_async_copy(buf.at[j], buf.at[j], sem.at[j]).wait()

        def issue_k_static(g, s, base_slot=0):
            issue_kv(k_hbm, g, s // 2, s % 2, s % NS)

        issue_wq(0)
        small = [
            pltpu.make_async_copy(ax_hbm, ax_s, small_sem.at[0]),
            pltpu.make_async_copy(b1_hbm, b1_s, small_sem.at[1]),
            pltpu.make_async_copy(b2_hbm, b2_s, small_sem.at[2]),
            pltpu.make_async_copy(gw_hbm, gw_s, small_sem.at[3]),
        ]
        for cp in small:
            cp.start()
        for t in range(1, D):
            issue_wq(t)
        for cp in small:
            cp.wait()

        ax = ax_s[...].astype(F32)
        gw = gw_s[...].astype(F32).reshape(1, D_MODEL)
        gate = jax.nn.sigmoid(jnp.sum(ax * gw, axis=-1, keepdims=True))
        ax8 = jnp.broadcast_to(ax, (8, D_MODEL))
        for kt in range(KT):
            xa_scr[kt] = ax8[:, kt * 128:(kt + 1) * 128]

        row = lax.broadcasted_iota(jnp.int32, (8, 128), 0)
        lane = lax.broadcasted_iota(jnp.int32, (8, 128), 1)

        def head_mask(tile_in_group):
            col = tile_in_group * 128 + lane
            return (col >= row * DH) & (col < (row + 1) * DH)

        def q_chunk(c, carry):
            def q_step(kt, acc):
                t = c * KT + kt
                wait_buf(wq_buf, wq_sem, t)
                tn = t + D

                @pl.when(tn < n_wq)
                def _():
                    issue_wq(tn)

                @pl.when(tn >= n_wq)
                def _():
                    issue_w1(tn - n_wq)
                lhs = xa_scr[kt].astype(BF16)
                return acc + jnp.dot(lhs, wq_buf[t], preferred_element_type=F32)
            acc = lax.fori_loop(0, KT, q_step, jnp.zeros((8, CW), F32))
            for i in range(CW // 128):
                tile = c * (CW // 128) + i
                tg = tile % NT_ if isinstance(tile, int) else lax.rem(tile, NT_)
                q_scr[tile] = jnp.where(head_mask(tg), acc[:, i * 128:(i + 1) * 128], 0.0)
            return carry
        lax.fori_loop(0, QC, q_chunk, 0)

        assert D <= KT + n_w2
        def w1_step(kt, acc):
            wait_buf(w1_buf, w1_sem, kt)
            tn = kt + D

            @pl.when(tn < KT)
            def _():
                issue_w1(tn)

            @pl.when((tn >= KT) & (tn < KT + n_w2))
            def _():
                issue_w(w2_hbm, w2_buf, w2_sem, tn - KT)
            if KT - 1 + D >= KT + n_w2:
                @pl.when(tn >= KT + n_w2)
                def _():
                    s = tn - KT - n_w2
                    issue_kv(k_hbm, 0, s // 2, s % 2, s)
            lhs = xa_scr[kt].astype(BF16)
            return acc + jnp.dot(lhs, w1_buf[kt], preferred_element_type=F32)
        hacc = lax.fori_loop(0, KT, w1_step, jnp.zeros((8, F), F32))
        b1 = b1_s[...].astype(F32).reshape(1, F)
        h = _gelu(hacc + b1)
        for j in range(n_w2):
            h_scr[j] = h[:, j * WB:(j + 1) * WB]

        def w2_step(j, acc):
            wait_buf(w2_buf, w2_sem, j)
            tn = j + D

            @pl.when(tn < n_w2)
            def _():
                issue_w(w2_hbm, w2_buf, w2_sem, tn)

            @pl.when(tn >= n_w2)
            def _():
                s = tn - n_w2
                issue_kv(k_hbm, 0, s // 2, s % 2, s)
            lhs = h_scr[j].astype(BF16)
            return acc + jnp.dot(lhs, w2_buf[j], preferred_element_type=F32)
        bacc = lax.fori_loop(0, n_w2, w2_step, jnp.zeros((8, D_MODEL), F32))
        b2 = b2_s[...].astype(F32).reshape(1, D_MODEL)
        bout = bacc[0:1, :] + b2

        HD = D // 2

        def group(g, carry):
            s_scr[...] = jnp.zeros(s_scr.shape, F32)

            def k_step(kt, carry):
                for c in range(2):
                    slot = (2 * kt + c) & (NS - 1)
                    wait_buf(ring, ring_sem, slot)
                    kn = kt + HD
                    nslot = (2 * kn + c) & (NS - 1)

                    @pl.when(kn < NT_)
                    def _():
                        issue_kv(k_hbm, g, kn, c, nslot)

                    @pl.when(kn >= NT_)
                    def _():
                        issue_kv(v_hbm, g, kn - NT_, c, nslot)
                    lhs = q_scr[g * NT_ + kt].astype(BF16)
                    s_scr[c] += jnp.dot(lhs, ring[slot], preferred_element_type=F32)
                return carry
            lax.fori_loop(0, NT_, k_step, 0)

            s0 = s_scr[0] * scale
            s1 = s_scr[1] * scale
            m = jnp.maximum(jnp.max(s0, axis=1, keepdims=True), jnp.max(s1, axis=1, keepdims=True))
            p0 = jnp.exp(s0 - m)
            p1 = jnp.exp(s1 - m)
            l = jnp.sum(p0, axis=1, keepdims=True) + jnp.sum(p1, axis=1, keepdims=True)
            p_scr[0] = p0.astype(BF16)
            p_scr[1] = p1.astype(BF16)
            il_scr[...] = jnp.broadcast_to(1.0 / l, (8, 128))

            def v_step(nt, carry):
                acc = jnp.zeros((8, 128), F32)
                for c in range(2):
                    slot = (2 * nt + c) & (NS - 1)
                    wait_buf(ring, ring_sem, slot)
                    nn = nt + HD
                    nslot = (2 * nn + c) & (NS - 1)

                    @pl.when(nn < NT_)
                    def _():
                        issue_kv(v_hbm, g, nn, c, nslot)

                    @pl.when((nn >= NT_) & (g + 1 < NG))
                    def _():
                        issue_kv(k_hbm, g + 1, nn - NT_, c, nslot)

                    @pl.when((nn >= NT_) & (g + 1 >= NG))
                    def _():
                        issue_w(wo_hbm, wo_buf, wo_sem, 2 * (nn - NT_) + c)
                    acc += lax.dot_general(p_scr[c], ring[slot], (((1,), (1,)), ((), ())),
                                           preferred_element_type=F32)
                o_scr[g * NT_ + nt] = jnp.where(head_mask(nt), acc * il_scr[...], 0.0)
                return carry
            lax.fori_loop(0, NT_, v_step, 0)
            return carry
        lax.fori_loop(0, NG, group, 0)

        def wo_step(j, acc):
            wait_buf(wo_buf, wo_sem, j)

            @pl.when(j + D < n_wo)
            def _():
                issue_w(wo_hbm, wo_buf, wo_sem, j + D)
            for i in range(WB // 128):
                lhs = o_scr[j * (WB // 128) + i].astype(BF16)
                acc += jnp.dot(lhs, wo_buf[j, pl.ds(i * 128, 128), :], preferred_element_type=F32)
            return acc
        aacc = lax.fori_loop(0, n_wo, wo_step, jnp.zeros((8, D_MODEL), F32))
        a = jnp.sum(aacc, axis=0, keepdims=True)
        out = gate * a + (1.0 - gate) * bout
        o_ref[...] = out.astype(o_ref.dtype)

    scratch = [
        pltpu.VMEM((NS, 128, CW), BF16),
        pltpu.VMEM((n_wq, 128, CW), BF16),
        pltpu.VMEM((KT, 128, F), BF16),
        pltpu.VMEM((n_w2, WB, D_MODEL), BF16),
        pltpu.VMEM((n_wo, WB, D_MODEL), BF16),
        pltpu.VMEM((1, D_MODEL), BF16),
        pltpu.VMEM((F,), BF16),
        pltpu.VMEM((D_MODEL,), BF16),
        pltpu.VMEM((D_MODEL,), BF16),
        pltpu.VMEM((KT, 8, 128), F32),
        pltpu.VMEM((HQ * DH // 128, 8, 128), F32),
        pltpu.VMEM((n_w2, 8, WB), F32),
        pltpu.VMEM((NC, 8, CW), F32),
        pltpu.VMEM((NC, 8, CW), BF16),
        pltpu.VMEM((HQ * DH // 128, 8, 128), F32),
        pltpu.VMEM((8, 128), F32),
        pltpu.SemaphoreType.DMA((NS,)),
        pltpu.SemaphoreType.DMA((n_wq,)),
        pltpu.SemaphoreType.DMA((KT,)),
        pltpu.SemaphoreType.DMA((n_w2,)),
        pltpu.SemaphoreType.DMA((n_wo,)),
        pltpu.SemaphoreType.DMA((4,)),
    ]
    return kernel, scratch


@jax.jit
def pallas_gated_mix__sliding_block_cached__dense_activation_gelu__decode_kernel(A_x, A_k_cache, A_v_cache, A_wq, A_wo, B_x, B_w1, B_b1, B_w2, B_b2, gate_w):
    _, _, D_MODEL = A_x.shape
    _, Hkv, Sk, Dh = A_k_cache.shape
    assert Hkv == HQ and Dh == DH
    W = min(4096, max(256, Sk // 4))
    F = B_w1.shape[1]
    kt = jnp.swapaxes(A_k_cache, 2, 3).reshape(HQ * DH, Sk)
    vt = jnp.swapaxes(A_v_cache, 2, 3).reshape(HQ * DH, Sk)
    kernel, scratch = make_kernel(Sk, W, D_MODEL, F, D=4, NS=8, pat='0111')
    out = pl.pallas_call(
        kernel,
        out_shape=jax.ShapeDtypeStruct((1, D_MODEL), A_x.dtype),
        in_specs=[pl.BlockSpec(memory_space=pl.ANY)] * 10,
        out_specs=pl.BlockSpec(memory_space=pltpu.VMEM),
        scratch_shapes=scratch,
        compiler_params=pltpu.CompilerParams(vmem_limit_bytes=64 * 1024 * 1024),
    )(A_x.reshape(1, D_MODEL), kt, vt, A_wq, A_wo, B_w1, B_b1, B_w2, B_b2, gate_w)
    return out.reshape(1, 1, D_MODEL)
```

```python
import functools
import jax
import jax.numpy as jnp
from jax import lax
import jax.experimental.pallas as pl
import jax.experimental.pallas.tpu as pltpu

HQ, DH = 32, 192
GH = 8
GR = GH * DH
NT_ = GR // 128
CW = 2048
JR = 8
F32, BF16 = jnp.float32, jnp.bfloat16


def make_kernel(Sk, W, D_MODEL, F, *, D=4, NS=8, pat="0111", patk=None, nocomp='', nobc=True, ng=None, smallprio=0):
    NG = HQ // GH if ng is None else ng
    NC = W // CW
    KT = D_MODEL // 128
    QC = HQ * DH // CW
    NB = 4
    n_wq = QC * NB
    n_w1 = NB
    n_w2 = NB
    W2R = F // (16 * NB)
    WOR = 32
    scale = DH ** -0.5
    patk = patk or pat
    assert NC == 2 and NS & (NS - 1) == 0 and NS > D and D <= 2 * NT_
    assert 24 % NS == 0 or NS == 16 or NS == 8

    def kernel(ax_hbm, k_hbm, v_hbm, wq_hbm, wo_hbm, w1_hbm, b1_hbm, w2_hbm, b2_hbm, gw_hbm,
               o_ref,
               ring, wq_buf, w1_buf, w2_buf, wo_buf,
               ax_s, b1_s, b2_s, gw_s,
               oacc_scr, q_scr, s_scr, p_scr, il_scr, acc_scr,
               ring_sem, wq_sem, w1_sem, w2_sem, wo_sem, small_sem):

        def prio(p, n):
            return int(p[n % len(p)])

        def kv_copies(src, g, rt, c, slot):
            cps = []
            for i in range(128 // JR):
                r0 = pl.multiple_of(g * GR + rt * 128 + i * JR, JR)
                c0 = pl.multiple_of(Sk - W + c * CW, CW)
                cps.append(pltpu.make_async_copy(src.at[pl.ds(r0, JR), pl.ds(c0, CW)],
                                                 ring.at[slot, pl.ds(i * JR, JR), :],
                                                 ring_sem.at[slot]))
            return cps

        def wo_copies(g, rt, c):
            cps = []
            nj = 128 // WOR // NC
            for i in range(nj):
                off = (c * nj + i) * WOR
                r0 = pl.multiple_of(g * GR + rt * 128 + off, WOR)
                cps.append(pltpu.make_async_copy(wo_hbm.at[pl.ds(r0, WOR), :],
                                                 wo_buf.at[g * NT_ + rt, pl.ds(pl.multiple_of(off, WOR), WOR), :],
                                                 wo_sem.at[rt]))
            return cps

        def issue_v(g, rt, c, slot):
            cps = kv_copies(v_hbm, g, rt, c, slot)
            wos = wo_copies(g, rt, c)
            order = []
            per = len(cps) // len(wos)
            for n, cp in enumerate(cps):
                order.append(cp)
                if n % per == per - 1:
                    order.append(wos[n // per])
            for n, cp in enumerate(order):
                cp.start(priority=prio(patk, n))

        def issue_k(g, rt, c, slot):
            for n, cp in enumerate(kv_copies(k_hbm, g, rt, c, slot)):
                cp.start(priority=prio(pat, n))

        def wq_copies(t):
            c = t // NB
            ib = t - c * NB
            cps = []
            for i in range(16 // NB):
                for kt in range(KT):
                    r0 = pl.multiple_of(kt * 128 + (ib * (16 // NB) + i) * JR, JR)
                    c0 = pl.multiple_of(c * CW, CW)
                    cps.append(pltpu.make_async_copy(wq_hbm.at[pl.ds(r0, JR), pl.ds(c0, CW)],
                                                     wq_buf.at[c, pl.ds(r0, JR), :],
                                                     wq_sem.at[t]))
            return cps

        def w1_copies(ib):
            cps = []
            for i in range(16 // NB):
                for kt in range(KT):
                    r0 = pl.multiple_of(kt * 128 + (ib * (16 // NB) + i) * JR, JR)
                    cps.append(pltpu.make_async_copy(w1_hbm.at[pl.ds(r0, JR), :],
                                                     w1_buf.at[pl.ds(r0, JR), :],
                                                     w1_sem.at[ib]))
            return cps

        def w2_copies(ib):
            cps = []
            for i in range(4):
                for q in range(4):
                    r0 = pl.multiple_of(q * (F // 4) + (ib * 4 + i) * W2R, 8)
                    cps.append(pltpu.make_async_copy(w2_hbm.at[pl.ds(r0, W2R), :],
                                                     w2_buf.at[pl.ds(r0, W2R), :],
                                                     w2_sem.at[ib]))
            return cps

        def start_all(cps):
            for n, cp in enumerate(cps):
                cp.start(priority=prio(pat, n))

        def wait_all(cps):
            for cp in cps:
                cp.wait()

        def wait_slot(slot):
            pltpu.make_async_copy(ring.at[slot], ring.at[slot], ring_sem.at[slot]).wait()

        phases = [
            ("wq", n_wq, lambda t: start_all(wq_copies(t))),
            ("w1", n_w1, lambda t: start_all(w1_copies(t))),
            ("w2", n_w2, lambda t: start_all(w2_copies(t))),
            ("k0", 2 * NT_, lambda s: issue_k(0, s // 2, s % 2, s & (NS - 1))),
        ]
        if NG == 0:
            phases = phases[:-1]
            if '1' in nocomp:
                phases = phases[:1]
        offs = {}
        o = 0
        for name, n, _ in phases:
            offs[name] = o
            o += n

        def issue_ahead(name, t):
            n_this = dict((a, b) for a, b, _ in phases)[name]
            lo, hi = offs[name] + D, offs[name] + n_this + D
            tg = offs[name] + t + D
            for qn, n, fn in phases:
                qlo, qhi = offs[qn], offs[qn] + n
                if max(lo, qlo) >= min(hi, qhi):
                    continue
                if lo >= qlo and hi <= qhi:
                    fn(tg - qlo)
                else:
                    @pl.when((tg >= qlo) & (tg < qhi))
                    def _(fn=fn, qlo=qlo):
                        fn(tg - qlo)

        assert D <= n_wq
        start_all(wq_copies(0))
        small = [
            pltpu.make_async_copy(ax_hbm, ax_s, small_sem.at[0]),
            pltpu.make_async_copy(b1_hbm, b1_s, small_sem.at[1]),
            pltpu.make_async_copy(b2_hbm, b2_s, small_sem.at[2]),
            pltpu.make_async_copy(gw_hbm, gw_s, small_sem.at[3]),
        ]
        if 's' in nocomp:
            small = []
        for cp in small:
            cp.start(priority=smallprio)
        for t in range(1, D):
            start_all(wq_copies(t))
        for cp in small:
            cp.wait()

        ax = ax_s[...].astype(F32)
        gw = gw_s[...].astype(F32).reshape(1, D_MODEL)
        gate = jax.nn.sigmoid(jnp.sum(ax * gw, axis=-1, keepdims=True))
        ax8 = jnp.broadcast_to(ax, (8, D_MODEL)).astype(BF16)

        row = lax.broadcasted_iota(jnp.int32, (8, 128), 0)
        lane = lax.broadcasted_iota(jnp.int32, (8, 128), 1)

        def head_mask(tile_in_group):
            col = tile_in_group * 128 + lane
            return (col >= row * DH) & (col < (row + 1) * DH)

        def q_step(t, carry):
            wait_all(wq_copies(t))
            issue_ahead("wq", t)

            @pl.when(t % NB == NB - 1)
            def _():
                c = t // NB
                if 'q' in nocomp:
                    acc = jnp.zeros((8, CW), F32)
                else:
                    acc = jnp.dot(ax8, wq_buf[c], preferred_element_type=F32)
                for i in range(CW // 128):
                    tile = c * (CW // 128) + i
                    q_scr[tile] = jnp.where(head_mask(lax.rem(tile, NT_)), acc[:, i * 128:(i + 1) * 128], 0.0)
            return carry
        lax.fori_loop(0, n_wq, q_step, 0)

        def w1_step(t, carry):
            wait_all(w1_copies(t))
            issue_ahead("w1", t)
            return carry
        if '1' not in nocomp: lax.fori_loop(0, n_w1, w1_step, 0)

        def w2_step(t, carry):
            wait_all(w2_copies(t))
            issue_ahead("w2", t)
            return carry
        if '1' not in nocomp: lax.fori_loop(0, n_w2, w2_step, 0)

        b1 = b1_s[...].astype(F32).reshape(1, F)
        b2 = b2_s[...].astype(F32).reshape(1, D_MODEL)
        if 'm' in nocomp:
            bout = b2
        else:
            h = jax.nn.gelu(jnp.dot(ax8, w1_buf[...], preferred_element_type=F32) + b1, approximate=True)
            bout = jnp.dot(h.astype(BF16), w2_buf[...], preferred_element_type=F32)[0:1, :] + b2
        acc_scr[...] = jnp.zeros(acc_scr.shape, F32)
        oacc_scr[...] = jnp.zeros((8, 128), F32)
        mlp = (1.0 - gate) * bout


        def k_body(g, s, nxt):
            kt, c = s >> 1, s & 1
            wait_slot(s & (NS - 1))
            nxt(s + D)
            if 'k' not in nocomp:
                lhs = q_scr[g * NT_ + kt].astype(BF16)
                s_scr[c] += jnp.dot(lhs, ring[s & (NS - 1)], preferred_element_type=F32)

        def v_body(g, s, nxt):
            nt, c = s >> 1, s & 1
            slot = (s + 2 * NT_) & (NS - 1)
            wait_slot(slot)
            nxt(s + D)
            if 'v' not in nocomp:
                oacc_scr[...] += lax.dot_general(p_scr[c], ring[slot], (((1,), (1,)), ((), ())),
                                                 preferred_element_type=F32)

            @pl.when(c == 1)
            def _():
                t = g * NT_ + nt
                pltpu.make_async_copy(wo_buf.at[t], wo_buf.at[t], wo_sem.at[nt]).wait()
                o = jnp.where(head_mask(nt), oacc_scr[...] * il_scr[...], 0.0).astype(BF16)
                oacc_scr[...] = jnp.zeros((8, 128), F32)
                if 'p' not in nocomp:
                    acc_scr[...] += jnp.dot(o, wo_buf[t], preferred_element_type=F32)

        def loop(lo, hi, body):
            def f(i, carry):
                body(i)
                return carry
            lax.fori_loop(lo, hi, f, 0)

        def group(g, carry):
            s_scr[...] = jnp.zeros(s_scr.shape, F32)
            NSTEP = 2 * NT_
            loop(0, NSTEP - D, lambda s: k_body(g, s, lambda sn: issue_k(g, sn >> 1, sn & 1, sn & (NS - 1))))
            loop(NSTEP - D, NSTEP, lambda s: k_body(
                g, s, lambda sn: issue_v(g, (sn - NSTEP) >> 1, sn & 1, sn & (NS - 1))))

            s0 = s_scr[0] * scale
            s1 = s_scr[1] * scale
            m = jnp.maximum(jnp.max(s0, axis=1, keepdims=True), jnp.max(s1, axis=1, keepdims=True))
            p0 = jnp.exp(s0 - m)
            p1 = jnp.exp(s1 - m)
            l = jnp.sum(p0, axis=1, keepdims=True) + jnp.sum(p1, axis=1, keepdims=True)
            p_scr[0] = p0.astype(BF16)
            p_scr[1] = p1.astype(BF16)
            il_scr[...] = jnp.broadcast_to(1.0 / l, (8, 128))

            loop(0, NSTEP - D, lambda s: v_body(
                g, s, lambda sn: issue_v(g, sn >> 1, sn & 1, (sn + NSTEP) & (NS - 1))))

            def cross(sn):
                @pl.when(g + 1 < NG)
                def _():
                    issue_k(g + 1, (sn - NSTEP) >> 1, sn & 1, (sn + NSTEP) & (NS - 1))
            loop(NSTEP - D, NSTEP, lambda s: v_body(g, s, cross))
            return carry
        lax.fori_loop(0, NG, group, 0)

        a = jnp.sum(acc_scr[...], axis=0, keepdims=True)
        o_ref[...] = (gate * a + mlp).astype(o_ref.dtype)

    scratch = [
        pltpu.VMEM((NS, 128, CW), BF16),
        pltpu.VMEM((QC, D_MODEL, CW), BF16),
        pltpu.VMEM((D_MODEL, F), BF16),
        pltpu.VMEM((F, D_MODEL), BF16),
        pltpu.VMEM((HQ * DH // 128, 128, D_MODEL), BF16),
        pltpu.VMEM((1, D_MODEL), BF16),
        pltpu.VMEM((F,), BF16),
        pltpu.VMEM((D_MODEL,), BF16),
        pltpu.VMEM((D_MODEL,), BF16),
        pltpu.VMEM((8, 128), F32),
        pltpu.VMEM((HQ * DH // 128, 8, 128), F32),
        pltpu.VMEM((NC, 8, CW), F32),
        pltpu.VMEM((NC, 8, CW), BF16),
        pltpu.VMEM((8, 128), F32),
        pltpu.VMEM((8, D_MODEL), F32),
        pltpu.SemaphoreType.DMA((NS,)),
        pltpu.SemaphoreType.DMA((n_wq,)),
        pltpu.SemaphoreType.DMA((n_w1,)),
        pltpu.SemaphoreType.DMA((n_w2,)),
        pltpu.SemaphoreType.DMA((NT_,)),
        pltpu.SemaphoreType.DMA((4,)),
    ]
    return kernel, scratch, nobc


@jax.jit
def pallas_gated_mix__sliding_block_cached__dense_activation_gelu__decode_kernel(A_x, A_k_cache, A_v_cache, A_wq, A_wo, B_x, B_w1, B_b1, B_w2, B_b2, gate_w):
    _, _, D_MODEL = A_x.shape
    _, Hkv, Sk, Dh = A_k_cache.shape
    assert Hkv == HQ and Dh == DH
    W = min(4096, max(256, Sk // 4))
    F = B_w1.shape[1]
    kt = jnp.swapaxes(A_k_cache, 2, 3).reshape(HQ * DH, Sk)
    vt = jnp.swapaxes(A_v_cache, 2, 3).reshape(HQ * DH, Sk)
    kernel, scratch, nobc = make_kernel(Sk, W, D_MODEL, F, D=6, NS=8, pat='01')
    out = pl.pallas_call(
        kernel,
        out_shape=jax.ShapeDtypeStruct((1, D_MODEL), A_x.dtype),
        in_specs=[pl.BlockSpec(memory_space=pl.ANY)] * 10,
        out_specs=pl.BlockSpec(memory_space=pltpu.VMEM),
        scratch_shapes=scratch,
        compiler_params=pltpu.CompilerParams(vmem_limit_bytes=64 * 1024 * 1024, disable_bounds_checks=nobc, disable_semaphore_checks=nobc),
    )(A_x.reshape(1, D_MODEL), kt, vt, A_wq, A_wo, B_w1, B_b1, B_w2, B_b2, gate_w)
    return out.reshape(1, 1, D_MODEL)
```

```python
import functools
import jax
import jax.numpy as jnp
from jax import lax
import jax.experimental.pallas as pl
import jax.experimental.pallas.tpu as pltpu

HQ, DH = 32, 192
GH = 8
GR = GH * DH
NT_ = GR // 128
CW = 2048
JR = 8
F32, BF16 = jnp.float32, jnp.bfloat16


def make_kernel(Sk, W, D_MODEL, F, *, D=4, NS=8, pat="0111", patk=None, nocomp='', nobc=True, ng=None, smallprio=0, KJR=8, KJC=2048, korder='rc', WOR=32, W2R=32, pad=0):
    NG = HQ // GH if ng is None else ng
    NC = W // CW
    KT = D_MODEL // 128
    QC = HQ * DH // CW
    NB = 4
    n_wq = QC * NB
    n_w1 = NB
    n_w2 = F // 256
    scale = DH ** -0.5
    patk = patk or pat
    assert NC == 2 and NS & (NS - 1) == 0 and NS > D and D <= 2 * NT_
    assert 24 % NS == 0 or NS == 16 or NS == 8

    def kernel(ax_hbm, k_hbm, v_hbm, wq_hbm, wo_hbm, w1_hbm, b1_hbm, w2_hbm, b2_hbm, gw_hbm,
               o_ref,
               *scr):
        if pad:
            scr = scr[1:]
        (ring, wq_buf, w1_buf, w2_buf, wo_buf,
               ax_s, b1_s, b2_s, gw_s,
               oacc_scr, h_scr, q_scr, s_scr, p_scr, il_scr, acc_scr,
               ring_sem, wq_sem, w1_sem, w2_sem, wo_sem, small_sem) = scr

        def prio(p, n):
            return int(p[n % len(p)])

        def kv_copies(src, g, rt, c, slot):
            cps = []
            na, nb = 128 // KJR, CW // KJC
            jobs = [(i, j) for i in range(na) for j in range(nb)] if korder == 'rc' else [(i, j) for j in range(nb) for i in range(na)]
            for i, j in jobs:
                r0 = pl.multiple_of(g * GR + rt * 128 + i * KJR, KJR)
                c0 = pl.multiple_of(Sk - W + c * CW + j * KJC, KJC)
                cps.append(pltpu.make_async_copy(src.at[pl.ds(r0, KJR), pl.ds(c0, KJC)],
                                                 ring.at[slot, pl.ds(i * KJR, KJR), pl.ds(j * KJC, KJC)],
                                                 ring_sem.at[slot]))
            return cps

        def wo_copies(g, rt, c):
            cps = []
            nj = 128 // WOR // NC
            for i in range(nj):
                off = (c * nj + i) * WOR
                r0 = pl.multiple_of(g * GR + rt * 128 + off, WOR)
                cps.append(pltpu.make_async_copy(wo_hbm.at[pl.ds(r0, WOR), :],
                                                 wo_buf.at[g * NT_ + rt, pl.ds(pl.multiple_of(off, WOR), WOR), :],
                                                 wo_sem.at[rt]))
            return cps

        def issue_v(g, rt, c, slot):
            cps = kv_copies(v_hbm, g, rt, c, slot)
            wos = wo_copies(g, rt, c)
            if 'w' in nocomp:
                for n, cp in enumerate(cps):
                    cp.start(priority=prio(patk, n))
                return
            order = []
            per = len(cps) // len(wos)
            for n, cp in enumerate(cps):
                order.append(cp)
                if n % per == per - 1:
                    order.append(wos[n // per])
            for n, cp in enumerate(order):
                cp.start(priority=prio(patk, n))

        def issue_k(g, rt, c, slot):
            for n, cp in enumerate(kv_copies(k_hbm, g, rt, c, slot)):
                cp.start(priority=prio(pat, n))

        def wq_copies(t):
            c = t // NB
            ib = t - c * NB
            cps = []
            for i in range(16 // NB):
                for kt in range(KT):
                    r0 = pl.multiple_of(kt * 128 + (ib * (16 // NB) + i) * JR, JR)
                    c0 = pl.multiple_of(c * CW, CW)
                    cps.append(pltpu.make_async_copy(wq_hbm.at[pl.ds(r0, JR), pl.ds(c0, CW)],
                                                     wq_buf.at[c, pl.ds(r0, JR), :],
                                                     wq_sem.at[t]))
            return cps

        def w1_copies(ib):
            cps = []
            for i in range(16 // NB):
                for kt in range(KT):
                    r0 = pl.multiple_of(kt * 128 + (ib * (16 // NB) + i) * JR, JR)
                    cps.append(pltpu.make_async_copy(w1_hbm.at[pl.ds(r0, JR), :],
                                                     w1_buf.at[pl.ds(r0, JR), :],
                                                     w1_sem.at[ib]))
            return cps

        def w2_copies(t):
            cps = []
            for i in range(128 // W2R):
                for h in range(2):
                    r0 = pl.multiple_of((t + h * n_w2) * 128 + i * W2R, W2R)
                    cps.append(pltpu.make_async_copy(w2_hbm.at[pl.ds(r0, W2R), :],
                                                     w2_buf.at[t, h, pl.ds(i * W2R, W2R), :],
                                                     w2_sem.at[t]))
            return cps

        def start_all(cps):
            for n, cp in enumerate(cps):
                cp.start(priority=prio(pat, n))

        def wait_all(cps):
            for cp in cps:
                cp.wait()

        def wait_slot(slot):
            pltpu.make_async_copy(ring.at[slot], ring.at[slot], ring_sem.at[slot]).wait()

        phases = [
            ("wq", n_wq, lambda t: start_all(wq_copies(t))),
            ("w1", n_w1, lambda t: start_all(w1_copies(t))),
            ("k0", 2 * NT_, lambda s: issue_k(0, s // 2, s % 2, s & (NS - 1))),
        ]
        if NG == 0:
            phases = phases[:-1]
            if '1' in nocomp:
                phases = phases[:1]
        offs = {}
        o = 0
        for name, n, _ in phases:
            offs[name] = o
            o += n

        def issue_ahead(name, t):
            n_this = dict((a, b) for a, b, _ in phases)[name]
            lo, hi = offs[name] + D, offs[name] + n_this + D
            tg = offs[name] + t + D
            for qn, n, fn in phases:
                qlo, qhi = offs[qn], offs[qn] + n
                if max(lo, qlo) >= min(hi, qhi):
                    continue
                if lo >= qlo and hi <= qhi:
                    fn(tg - qlo)
                else:
                    @pl.when((tg >= qlo) & (tg < qhi))
                    def _(fn=fn, qlo=qlo):
                        fn(tg - qlo)

        assert D <= n_wq
        start_all(wq_copies(0))
        small = [
            pltpu.make_async_copy(ax_hbm, ax_s, small_sem.at[0]),
            pltpu.make_async_copy(b1_hbm, b1_s, small_sem.at[1]),
            pltpu.make_async_copy(b2_hbm, b2_s, small_sem.at[2]),
            pltpu.make_async_copy(gw_hbm, gw_s, small_sem.at[3]),
        ]
        if 's' in nocomp:
            small = []
        for cp in small:
            cp.start(priority=smallprio)
        for t in range(1, D):
            start_all(wq_copies(t))
        for cp in small:
            cp.wait()

        ax = ax_s[...].astype(F32)
        gw = gw_s[...].astype(F32).reshape(1, D_MODEL)
        gate = jax.nn.sigmoid(jnp.sum(ax * gw, axis=-1, keepdims=True))
        ax8 = jnp.broadcast_to(ax, (8, D_MODEL)).astype(BF16)

        row = lax.broadcasted_iota(jnp.int32, (8, 128), 0)
        lane = lax.broadcasted_iota(jnp.int32, (8, 128), 1)

        def head_mask(tile_in_group):
            col = tile_in_group * 128 + lane
            return (col >= row * DH) & (col < (row + 1) * DH)

        def q_step(t, carry):
            wait_all(wq_copies(t))
            issue_ahead("wq", t)

            @pl.when(t % NB == NB - 1)
            def _():
                c = t // NB
                if 'q' in nocomp:
                    acc = jnp.zeros((8, CW), F32)
                else:
                    acc = jnp.dot(ax8, wq_buf[c], preferred_element_type=F32)
                for i in range(CW // 128):
                    tile = c * (CW // 128) + i
                    q_scr[tile] = jnp.where(head_mask(lax.rem(tile, NT_)), acc[:, i * 128:(i + 1) * 128], 0.0)
            return carry
        lax.fori_loop(0, n_wq, q_step, 0)

        def w1_step(t, carry):
            wait_all(w1_copies(t))
            issue_ahead("w1", t)
            return carry
        lax.fori_loop(0, n_w1, w1_step, 0)

        b1 = b1_s[...].astype(F32).reshape(1, F)
        if 'm' in nocomp:
            h = jnp.broadcast_to(b1, (8, F))
        else:
            h = jax.nn.gelu(jnp.dot(ax8, w1_buf[...], preferred_element_type=F32) + b1, approximate=True)
        for j in range(F // 128):
            h_scr[j] = h[:, j * 128:(j + 1) * 128]
        acc_scr[...] = jnp.zeros(acc_scr.shape, F32)
        oacc_scr[...] = jnp.zeros((8, 128), F32)


        def k_body(g, s, nxt):
            kt, c = s >> 1, s & 1
            wait_slot(s & (NS - 1))
            nxt(s + D)
            if 'k' not in nocomp:
                lhs = q_scr[g * NT_ + kt].astype(BF16)
                s_scr[c] += jnp.dot(lhs, ring[s & (NS - 1)], preferred_element_type=F32)

        def v_body(g, s, nxt):
            nt, c = s >> 1, s & 1
            slot = (s + 2 * NT_) & (NS - 1)
            wait_slot(slot)
            nxt(s + D)
            if 'v' not in nocomp:
                oacc_scr[...] += lax.dot_general(p_scr[c], ring[slot], (((1,), (1,)), ((), ())),
                                                 preferred_element_type=F32)

            @pl.when(c == 1)
            def _():
                t = g * NT_ + nt
                if 'w' not in nocomp:
                    pltpu.make_async_copy(wo_buf.at[t], wo_buf.at[t], wo_sem.at[nt]).wait()
                o = jnp.where(head_mask(nt), oacc_scr[...] * il_scr[...], 0.0).astype(BF16)
                oacc_scr[...] = jnp.zeros((8, 128), F32)
                if 'p' not in nocomp:
                    acc_scr[...] += jnp.dot(o, wo_buf[t], preferred_element_type=F32)

        def loop(lo, hi, body):
            def f(i, carry):
                body(i)
                return carry
            lax.fori_loop(lo, hi, f, 0)

        def group(g, carry):
            s_scr[...] = jnp.zeros(s_scr.shape, F32)
            NSTEP = 2 * NT_
            loop(0, NSTEP - D, lambda s: k_body(g, s, lambda sn: issue_k(g, sn >> 1, sn & 1, sn & (NS - 1))))
            loop(NSTEP - D, NSTEP, lambda s: k_body(
                g, s, lambda sn: issue_v(g, (sn - NSTEP) >> 1, sn & 1, sn & (NS - 1))))

            s0 = s_scr[0] * scale
            s1 = s_scr[1] * scale
            m = jnp.maximum(jnp.max(s0, axis=1, keepdims=True), jnp.max(s1, axis=1, keepdims=True))
            p0 = jnp.exp(s0 - m)
            p1 = jnp.exp(s1 - m)
            l = jnp.sum(p0, axis=1, keepdims=True) + jnp.sum(p1, axis=1, keepdims=True)
            p_scr[0] = p0.astype(BF16)
            p_scr[1] = p1.astype(BF16)
            il_scr[...] = jnp.broadcast_to(1.0 / l, (8, 128))

            loop(0, NSTEP - D, lambda s: v_body(
                g, s, lambda sn: issue_v(g, sn >> 1, sn & 1, (sn + NSTEP) & (NS - 1))))

            def cross(sn):
                @pl.when(g + 1 < NG)
                def _():
                    issue_k(g + 1, (sn - NSTEP) >> 1, sn & 1, (sn + NSTEP) & (NS - 1))

                @pl.when((g + 1 >= NG) & (sn - NSTEP < n_w2))
                def _():
                    start_all(w2_copies(sn - NSTEP))
            loop(NSTEP - D, NSTEP, lambda s: v_body(g, s, cross))
            return carry
        lax.fori_loop(0, NG, group, 0)

        b2 = b2_s[...].astype(F32).reshape(1, D_MODEL)
        base = gate * jnp.sum(acc_scr[...], axis=0, keepdims=True) + (1.0 - gate) * b2

        def w2_step(t, acc):
            pltpu.make_async_copy(w2_buf.at[t], w2_buf.at[t], w2_sem.at[t]).wait()
            if D < n_w2:
                @pl.when(t + D < n_w2)
                def _():
                    start_all(w2_copies(t + D))
            if 'm' not in nocomp:
                for hh in range(2):
                    acc += jnp.dot(h_scr[t + hh * n_w2].astype(BF16), w2_buf[t, hh], preferred_element_type=F32)
            return acc
        bacc = lax.fori_loop(0, n_w2, w2_step, jnp.zeros((8, D_MODEL), F32))
        o_ref[...] = (base + (1.0 - gate) * bacc[0:1, :]).astype(o_ref.dtype)

    scratch = ([pltpu.VMEM((pad * 2, 128), F32)] if pad else []) + [
        pltpu.VMEM((NS, 128, CW), BF16),
        pltpu.VMEM((QC, D_MODEL, CW), BF16),
        pltpu.VMEM((D_MODEL, F), BF16),
        pltpu.VMEM((n_w2, 2, 128, D_MODEL), BF16),
        pltpu.VMEM((HQ * DH // 128, 128, D_MODEL), BF16),
        pltpu.VMEM((1, D_MODEL), BF16),
        pltpu.VMEM((F,), BF16),
        pltpu.VMEM((D_MODEL,), BF16),
        pltpu.VMEM((D_MODEL,), BF16),
        pltpu.VMEM((8, 128), F32),
        pltpu.VMEM((F // 128, 8, 128), F32),
        pltpu.VMEM((HQ * DH // 128, 8, 128), F32),
        pltpu.VMEM((NC, 8, CW), F32),
        pltpu.VMEM((NC, 8, CW), BF16),
        pltpu.VMEM((8, 128), F32),
        pltpu.VMEM((8, D_MODEL), F32),
        pltpu.SemaphoreType.DMA((NS,)),
        pltpu.SemaphoreType.DMA((n_wq,)),
        pltpu.SemaphoreType.DMA((n_w1,)),
        pltpu.SemaphoreType.DMA((n_w2,)),
        pltpu.SemaphoreType.DMA((NT_,)),
        pltpu.SemaphoreType.DMA((4,)),
    ]
    return kernel, scratch, nobc


@jax.jit
def pallas_gated_mix__sliding_block_cached__dense_activation_gelu__decode_kernel(A_x, A_k_cache, A_v_cache, A_wq, A_wo, B_x, B_w1, B_b1, B_w2, B_b2, gate_w):
    _, _, D_MODEL = A_x.shape
    _, Hkv, Sk, Dh = A_k_cache.shape
    assert Hkv == HQ and Dh == DH
    W = min(4096, max(256, Sk // 4))
    F = B_w1.shape[1]
    kt = jnp.swapaxes(A_k_cache, 2, 3).reshape(HQ * DH, Sk)
    vt = jnp.swapaxes(A_v_cache, 2, 3).reshape(HQ * DH, Sk)
    kernel, scratch, nobc = make_kernel(Sk, W, D_MODEL, F, D=6, NS=8, pat='10')
    out = pl.pallas_call(
        kernel,
        out_shape=jax.ShapeDtypeStruct((1, D_MODEL), A_x.dtype),
        in_specs=[pl.BlockSpec(memory_space=pl.ANY)] * 10,
        out_specs=pl.BlockSpec(memory_space=pltpu.VMEM),
        scratch_shapes=scratch,
        compiler_params=pltpu.CompilerParams(vmem_limit_bytes=64 * 1024 * 1024, disable_bounds_checks=nobc, disable_semaphore_checks=nobc),
    )(A_x.reshape(1, D_MODEL), kt, vt, A_wq, A_wo, B_w1, B_b1, B_w2, B_b2, gate_w)
    return out.reshape(1, 1, D_MODEL)
```

```python
import jax
import jax.numpy as jnp
from jax import lax
import jax.experimental.pallas as pl
import jax.experimental.pallas.tpu as pltpu

HQ, DH = 32, 192
GH = 8
GR = GH * DH
NT = GR // 128
CW = 2048
JR = 8
NB = 4
WR = 32
LOOKAHEAD = 6
NS = 8
F32, BF16 = jnp.float32, jnp.bfloat16


def _start_all(copies):
    for n, cp in enumerate(copies):
        cp.start(priority=(n + 1) % 2)


def _wait_all(copies):
    for cp in copies:
        cp.wait()


def _loop(lo, hi, body):
    def f(i, carry):
        body(i)
        return carry
    lax.fori_loop(lo, hi, f, 0)


def _make_kernel(Sk, W, DM, F):
    D = LOOKAHEAD
    NG = HQ // GH
    NC = W // CW
    KT = DM // 128
    QC = HQ * DH // CW
    NSTEP = NT * NC
    n_wq, n_w1, n_w2 = QC * NB, NB, F // 256
    scale = DH ** -0.5
    assert NC == 2 and W % CW == 0 and (Sk - W) % CW == 0 and (HQ * DH) % CW == 0
    assert DM % 128 == 0 and F % 256 == 0 and NSTEP % NS == 0
    assert n_w2 <= D <= min(n_wq, NS - 1)

    def kernel(x_hbm, k_hbm, v_hbm, wq_hbm, wo_hbm, w1_hbm, b1_hbm, w2_hbm, b2_hbm, gw_hbm,
               o_ref,
               ring, wq_buf, w1_buf, w2_buf, wo_buf, x_s, b1_s, b2_s, gw_s,
               q_scr, s_scr, p_scr, il_scr, o_scr, h_scr, acc_scr,
               ring_sem, wq_sem, w1_sem, w2_sem, wo_sem, small_sem):

        def kv_copies(src, g, s, slot):
            rt, c = s >> 1, s & 1
            c0 = pl.multiple_of(Sk - W + c * CW, CW)
            return [pltpu.make_async_copy(
                src.at[pl.ds(pl.multiple_of(g * GR + rt * 128 + i * JR, JR), JR), pl.ds(c0, CW)],
                ring.at[slot, pl.ds(i * JR, JR), :], ring_sem.at[slot]) for i in range(128 // JR)]

        def wo_copies(g, s):
            rt, c = s >> 1, s & 1
            nj = 128 // WR // NC
            cps = []
            for i in range(nj):
                off = pl.multiple_of((c * nj + i) * WR, WR)
                cps.append(pltpu.make_async_copy(
                    wo_hbm.at[pl.ds(pl.multiple_of(g * GR + rt * 128 + off, WR), WR), :],
                    wo_buf.at[g * NT + rt, pl.ds(off, WR), :], wo_sem.at[rt]))
            return cps

        def issue_k(g, s, slot):
            _start_all(kv_copies(k_hbm, g, s, slot))

        def issue_v(g, s, slot):
            vs, wos = kv_copies(v_hbm, g, s, slot), wo_copies(g, s)
            per = len(vs) // len(wos)
            order = []
            for n, cp in enumerate(vs):
                order.append(cp)
                if n % per == per - 1:
                    order.append(wos[n // per])
            _start_all(order)

        def strided_rows(ib):
            return [pl.multiple_of(kt * 128 + (ib * (16 // NB) + i) * JR, JR)
                    for i in range(16 // NB) for kt in range(KT)]

        def wq_copies(t):
            c = t // NB
            c0 = pl.multiple_of(c * CW, CW)
            return [pltpu.make_async_copy(wq_hbm.at[pl.ds(r0, JR), pl.ds(c0, CW)],
                                          wq_buf.at[c, pl.ds(r0, JR), :], wq_sem.at[t])
                    for r0 in strided_rows(t - c * NB)]

        def w1_copies(t):
            return [pltpu.make_async_copy(w1_hbm.at[pl.ds(r0, JR), :], w1_buf.at[pl.ds(r0, JR), :], w1_sem.at[t])
                    for r0 in strided_rows(t)]

        def w2_copies(t):
            return [pltpu.make_async_copy(
                w2_hbm.at[pl.ds(pl.multiple_of((t + h * n_w2) * 128 + i * WR, WR), WR), :],
                w2_buf.at[t, h, pl.ds(i * WR, WR), :], w2_sem.at[t])
                for i in range(128 // WR) for h in range(2)]

        def wait_full(buf, sem, i):
            pltpu.make_async_copy(buf.at[i], buf.at[i], sem.at[i]).wait()

        phases = [(n_wq, lambda t: _start_all(wq_copies(t))),
                  (n_w1, lambda t: _start_all(w1_copies(t))),
                  (NSTEP, lambda s: issue_k(0, s, s & (NS - 1)))]

        def issue_ahead(phase, t):
            first = sum(n for n, _ in phases[:phase])
            lo, hi = first + D, first + phases[phase][0] + D
            tg = first + t + D
            start = 0
            for n, fn in phases:
                if lo >= start and hi <= start + n:
                    fn(tg - start)
                elif max(lo, start) < min(hi, start + n):
                    @pl.when((tg >= start) & (tg < start + n))
                    def _(fn=fn, start=start):
                        fn(tg - start)
                start += n

        small = [pltpu.make_async_copy(src, dst, small_sem.at[i]) for i, (src, dst) in enumerate(
            [(x_hbm, x_s), (b1_hbm, b1_s), (b2_hbm, b2_s), (gw_hbm, gw_s)])]
        _start_all(wq_copies(0))
        for cp in small:
            cp.start()
        for t in range(1, D):
            _start_all(wq_copies(t))
        _wait_all(small)

        x = x_s[...].astype(F32)
        gw = gw_s[...].astype(F32).reshape(1, DM)
        gate = jax.nn.sigmoid(jnp.sum(x * gw, axis=-1, keepdims=True))
        x8 = jnp.broadcast_to(x, (GH, DM)).astype(BF16)

        row = lax.broadcasted_iota(jnp.int32, (GH, 128), 0)
        lane = lax.broadcasted_iota(jnp.int32, (GH, 128), 1)

        def head_mask(tile):
            col = tile * 128 + lane
            return (col >= row * DH) & (col < (row + 1) * DH)

        def q_step(t):
            _wait_all(wq_copies(t))
            issue_ahead(0, t)

            @pl.when(t % NB == NB - 1)
            def _():
                c = t // NB
                q = jnp.dot(x8, wq_buf[c], preferred_element_type=F32)
                for i in range(CW // 128):
                    tile = c * (CW // 128) + i
                    q_scr[tile] = jnp.where(head_mask(lax.rem(tile, NT)), q[:, i * 128:(i + 1) * 128], 0.0)
        _loop(0, n_wq, q_step)

        def w1_step(t):
            _wait_all(w1_copies(t))
            issue_ahead(1, t)
        _loop(0, n_w1, w1_step)

        b1 = b1_s[...].astype(F32).reshape(1, F)
        h = jax.nn.gelu(jnp.dot(x8, w1_buf[...], preferred_element_type=F32) + b1, approximate=True)
        for j in range(F // 128):
            h_scr[j] = h[:, j * 128:(j + 1) * 128]
        acc_scr[...] = jnp.zeros(acc_scr.shape, F32)
        o_scr[...] = jnp.zeros(o_scr.shape, F32)

        def k_step(g, s, issue):
            slot = s & (NS - 1)
            wait_full(ring, ring_sem, slot)
            issue(s + D)
            q = q_scr[g * NT + (s >> 1)].astype(BF16)
            s_scr[s & 1] += jnp.dot(q, ring[slot], preferred_element_type=F32)

        def v_step(g, s, issue):
            nt, c = s >> 1, s & 1
            slot = (s + NSTEP) & (NS - 1)
            wait_full(ring, ring_sem, slot)
            issue(s + D)
            o_scr[...] += lax.dot_general(p_scr[c], ring[slot], (((1,), (1,)), ((), ())),
                                          preferred_element_type=F32)

            @pl.when(c == NC - 1)
            def _():
                t = g * NT + nt
                pltpu.make_async_copy(wo_buf.at[t], wo_buf.at[t], wo_sem.at[nt]).wait()
                o = jnp.where(head_mask(nt), o_scr[...] * il_scr[...], 0.0).astype(BF16)
                o_scr[...] = jnp.zeros(o_scr.shape, F32)
                acc_scr[...] += jnp.dot(o, wo_buf[t], preferred_element_type=F32)

        def group(g):
            s_scr[...] = jnp.zeros(s_scr.shape, F32)
            _loop(0, NSTEP - D, lambda s: k_step(g, s, lambda sn: issue_k(g, sn, sn & (NS - 1))))
            _loop(NSTEP - D, NSTEP, lambda s: k_step(
                g, s, lambda sn: issue_v(g, sn - NSTEP, sn & (NS - 1))))

            s0, s1 = s_scr[0] * scale, s_scr[1] * scale
            m = jnp.maximum(jnp.max(s0, axis=1, keepdims=True), jnp.max(s1, axis=1, keepdims=True))
            p0, p1 = jnp.exp(s0 - m), jnp.exp(s1 - m)
            l = jnp.sum(p0, axis=1, keepdims=True) + jnp.sum(p1, axis=1, keepdims=True)
            p_scr[0] = p0.astype(BF16)
            p_scr[1] = p1.astype(BF16)
            il_scr[...] = jnp.broadcast_to(1.0 / l, il_scr.shape)

            def issue_next_group(sn):
                @pl.when(g + 1 < NG)
                def _():
                    issue_k(g + 1, sn - NSTEP, (sn + NSTEP) & (NS - 1))

                @pl.when((g + 1 >= NG) & (sn - NSTEP < n_w2))
                def _():
                    _start_all(w2_copies(sn - NSTEP))

            _loop(0, NSTEP - D, lambda s: v_step(
                g, s, lambda sn: issue_v(g, sn, (sn + NSTEP) & (NS - 1))))
            _loop(NSTEP - D, NSTEP, lambda s: v_step(g, s, issue_next_group))
        _loop(0, NG, group)

        b2 = b2_s[...].astype(F32).reshape(1, DM)
        base = gate * jnp.sum(acc_scr[...], axis=0, keepdims=True) + (1.0 - gate) * b2

        def w2_step(t, acc):
            wait_full(w2_buf, w2_sem, t)
            for hh in range(2):
                acc += jnp.dot(h_scr[t + hh * n_w2].astype(BF16), w2_buf[t, hh], preferred_element_type=F32)
            return acc
        mlp = lax.fori_loop(0, n_w2, w2_step, jnp.zeros((GH, DM), F32))
        o_ref[...] = (base + (1.0 - gate) * mlp[0:1, :]).astype(o_ref.dtype)

    scratch = [
        pltpu.VMEM((NS, 128, CW), BF16),
        pltpu.VMEM((QC, DM, CW), BF16),
        pltpu.VMEM((DM, F), BF16),
        pltpu.VMEM((n_w2, 2, 128, DM), BF16),
        pltpu.VMEM((HQ * DH // 128, 128, DM), BF16),
        pltpu.VMEM((1, DM), BF16),
        pltpu.VMEM((F,), BF16),
        pltpu.VMEM((DM,), BF16),
        pltpu.VMEM((DM,), BF16),
        pltpu.VMEM((HQ * DH // 128, GH, 128), F32),
        pltpu.VMEM((NC, GH, CW), F32),
        pltpu.VMEM((NC, GH, CW), BF16),
        pltpu.VMEM((GH, 128), F32),
        pltpu.VMEM((GH, 128), F32),
        pltpu.VMEM((F // 128, GH, 128), F32),
        pltpu.VMEM((GH, DM), F32),
        pltpu.SemaphoreType.DMA((NS,)),
        pltpu.SemaphoreType.DMA((n_wq,)),
        pltpu.SemaphoreType.DMA((n_w1,)),
        pltpu.SemaphoreType.DMA((n_w2,)),
        pltpu.SemaphoreType.DMA((NT,)),
        pltpu.SemaphoreType.DMA((4,)),
    ]
    return kernel, scratch


@jax.jit
def pallas_gated_mix__sliding_block_cached__dense_activation_gelu__decode_kernel(
    A_x: jax.Array,
    A_k_cache: jax.Array,
    A_v_cache: jax.Array,
    A_wq: jax.Array,
    A_wo: jax.Array,
    B_x: jax.Array,
    B_w1: jax.Array,
    B_b1: jax.Array,
    B_w2: jax.Array,
    B_b2: jax.Array,
    gate_w: jax.Array,
):
    del B_x
    batch, sq, dm = A_x.shape
    _, hkv, sk, dh = A_k_cache.shape
    assert batch == 1 and sq == 1 and hkv == HQ and dh == DH
    w = min(4096, max(256, sk // 4))
    f = B_w1.shape[1]
    kt = jnp.swapaxes(A_k_cache, 2, 3).reshape(HQ * DH, sk)
    vt = jnp.swapaxes(A_v_cache, 2, 3).reshape(HQ * DH, sk)
    kernel, scratch = _make_kernel(sk, w, dm, f)
    out = pl.pallas_call(
        kernel,
        out_shape=jax.ShapeDtypeStruct((1, dm), A_x.dtype),
        in_specs=[pl.BlockSpec(memory_space=pl.ANY)] * 10,
        out_specs=pl.BlockSpec(memory_space=pltpu.VMEM),
        scratch_shapes=scratch,
        compiler_params=pltpu.CompilerParams(
            vmem_limit_bytes=64 * 1024 * 1024,
            disable_bounds_checks=True,
            disable_semaphore_checks=True,
        ),
    )(A_x.reshape(1, dm), kt, vt, A_wq, A_wo, B_w1, B_b1, B_w2, B_b2, gate_w)
    return out.reshape(1, 1, dm)
```
